```python
import jax
import jax.numpy as jnp

def _softmax(x, axis=-1):
    return jax.nn.softmax(x, axis=axis)

def _gelu(x):
    return jax.nn.gelu(x, approximate=True)

def _silu(x):
    return jax.nn.silu(x)

def _sigmoid(x):
    return jax.nn.sigmoid(x)

def _layernorm(x, axis=-1, eps=1e-05):
    m = jnp.mean(x, axis=axis, keepdims=True)
    v = jnp.var(x, axis=axis, keepdims=True)
    return (x - m) / jnp.sqrt(v + eps)

def _scatter_add(tgt, idx, src, axis=0):
    return tgt.at[idx].add(src)

def _segment_sum(src, seg, n):
    return jax.ops.segment_sum(src, seg, n)

class _Rng:

    def __init__(self, key):
        self._k = key

    def _next(self):
        self._k, sub = jax.random.split(self._k)
        return sub

    def normal(self, shape):
        return jax.random.normal(self._next(), shape, dtype=jnp.bfloat16)

    def randint(self, lo, hi, shape):
        return jax.random.randint(self._next(), shape, lo, hi, dtype=jnp.int32)

    def uniform(self, shape, lo=0.0, hi=1.0):
        return jax.random.uniform(self._next(), shape, jnp.bfloat16, lo, hi)

    def permutation(self, n):
        return jax.random.permutation(self._next(), n)
kernel_name = 'adaLN_cond__sliding_block_cached__mixer_s_mlp__decode'

def setup_inputs():
    _rng = _Rng(jax.random.key(int.from_bytes(__import__("os").urandom(4), "little")))
    _w = lambda a: (lambda t: t.astype(jnp.bfloat16) if jnp.issubdtype(t.dtype, jnp.floating) else t)(jnp.asarray(a))

    def _A_setup():
        B, Sq, D = (1, 1, 448)
        Hq, Hkv, Sk, Dh = (16, 8, 65536, 256)
        assert Hq % Hkv == 0, (Hq, Hkv)
        return {'x': _w((lambda *s: _rng.normal(s) * 0.05)(B, Sq, D)), 'k_cache': _w((lambda *s: _rng.normal(s) * 0.05)(B, Hkv, Sk, Dh)), 'v_cache': _w((lambda *s: _rng.normal(s) * 0.05)(B, Hkv, Sk, Dh)), 'wq': _w((lambda *s: _rng.normal(s) * 0.05)(D, Hq * Dh) * D ** (-0.5)), 'wo': _w((lambda *s: _rng.normal(s) * 0.05)(Hq * Dh, D) * (Hq * Dh) ** (-0.5))}
    _A_in = _A_setup()

    def _B_setup():
        B, S, D, F = (1, 1, 448, 1792)
        return {'x': _w((lambda *s: _rng.normal(s) * 0.05)(B, S, D)), 'w1': _w((lambda *s: _rng.normal(s) * 0.05)(D, D) * D ** (-0.5)), 'w2': _w((lambda *s: _rng.normal(s) * 0.05)(D, D) * D ** (-0.5)), 'w3': _w((lambda *s: _rng.normal(s) * 0.05)(D, F) * D ** (-0.5)), 'w4': _w((lambda *s: _rng.normal(s) * 0.05)(F, D) * F ** (-0.5))}
    _B_in = _B_setup()
    return {'A_x': _A_in['x'], 'A_k_cache': _A_in['k_cache'], 'A_v_cache': _A_in['v_cache'], 'A_wq': _A_in['wq'], 'A_wo': _A_in['wo'], 'B_x': _B_in['x'], 'B_w1': _B_in['w1'], 'B_w2': _B_in['w2'], 'B_w3': _B_in['w3'], 'B_w4': _B_in['w4'], 'c': _w((lambda *s: _rng.normal(s) * 0.05)(1, 448)), 'w_mod': _w((lambda *s: _rng.normal(s) * 0.05)(448, 6 * 448) * 448 ** (-0.5))}

def reference(A_x, A_k_cache, A_v_cache, A_wq, A_wo, B_x, B_w1, B_w2, B_w3, B_w4, c, w_mod):

    def _A_ref(x, k_cache, v_cache, wq, wo):
        B, Sq, D = x.shape
        Hq, Dh = (16, 256)
        Hkv, Sk = (k_cache.shape[1], k_cache.shape[2])
        W = min(4096, max(256, Sk // 4))
        rep = Hq // Hkv
        q = (lambda x, *d: x.transpose(*d))((x @ wq).reshape(B, Sq, Hq, Dh), 0, 2, 1, 3)
        k = jnp.repeat(k_cache[:, :, Sk - W:, :], rep, axis=1)
        v = jnp.repeat(v_cache[:, :, Sk - W:, :], rep, axis=1)
        scores = jnp.einsum('bhqd,bhkd->bhqk', q, k) * Dh ** (-0.5)
        p = _softmax(scores, axis=-1)
        o = jnp.einsum('bhqk,bhkd->bhqd', p, v)
        return (lambda x, *d: x.transpose(*d))(o, 0, 2, 1, 3).reshape(B, Sq, Hq * Dh) @ wo

    def _B_ref(x, w1, w2, w3, w4):
        B, S, D = x.shape
        h = _gelu(_layernorm(x, axis=-1) @ w1)
        c = D // 4
        g0 = jnp.pad(h[:, :, 0 * c:1 * c], ((0, 0), (1, 0), (0, 0)))[:, :S, :]
        g1 = jnp.pad(h[:, :, 1 * c:2 * c], ((0, 0), (0, 1), (0, 0)))[:, 1:, :]
        g2 = jnp.pad(h[:, :, 2 * c:3 * c], ((0, 0), (2, 0), (0, 0)))[:, :S, :]
        g3 = jnp.pad(h[:, :, 3 * c:], ((0, 0), (0, 2), (0, 0)))[:, 2:, :]
        hs = jnp.concatenate([g0, g1, g2, g3], axis=-1) @ w2
        x1 = x + hs
        h2 = _gelu(_layernorm(x1, axis=-1) @ w3) @ w4
        return x1 + h2
    x = A_x
    mod = (_silu(c) @ w_mod).reshape(c.shape[0], 6, 1, -1)
    sa, ca, ga, sb, cb, gb = (mod[:, 0].copy(), mod[:, 1].copy(), mod[:, 2].copy(), mod[:, 3].copy(), mod[:, 4].copy(), mod[:, 5].copy())
    h = _layernorm(x, axis=-1) * (1 + ca) + sa
    x = x + ga * _A_ref(h, A_k_cache, A_v_cache, A_wq, A_wo)
    h = _layernorm(x, axis=-1) * (1 + cb) + sb
    x = x + gb * _B_ref(h, B_w1, B_w2, B_w3, B_w4)
    return x
```

```python
import jax
import jax.numpy as jnp
from jax import lax
from jax.experimental import pallas as pl
from jax.experimental.pallas import tpu as pltpu

D, F = 448, 1792
HQ, HKV, DH = 16, 8, 256
WINDOW = 4096
EPS = 1e-5
ROWS = 8
LATE = 2304
BF16, F32 = jnp.bfloat16, jnp.float32

S_X, S_C, S_WM, S_WQ, S_WO, S_W3, S_K, S_V, S_W4, S_GATE = 0, 1, 2, 3, 4, 5, 6, 14, 22, 25
W4_BLOCKS = ((0, 256), (256, 128), (384, 64))
GATE_BLOCKS = ((0, 128), (128, 64), (192, 32))
WM_CUTS = ((4, 4, 4, 4, 2), (3, 4, 4, 4, 3), (2, 4, 4, 4, 4), (1, 4, 4, 4, 4, 1))
FF_CUTS = ((4, 4, 4, 2), (2, 4, 4, 4))
CFG = dict(phases=(0, 8, 31, 7), w3rows=16, share=3, end3=((7, 7), (7, 7)), end4=((14,), (14,)), mix=16, lead=20, grows=8,
           at=(55, 62), compute=True, wst=2, gshare=3)


def _layernorm(x):
    d = x - jnp.sum(x, axis=-1, keepdims=True) * (1.0 / D)
    return d * lax.rsqrt(jnp.sum(d * d, axis=-1, keepdims=True) * (1.0 / D) + EPS)


def _dot(a, b):
    return lax.dot_general(a, b, (((1,), (0,)), ((), ())), preferred_element_type=F32)


def _dot_t(a, b):
    return lax.dot_general(a, b, (((1,), (1,)), ((), ())), preferred_element_type=F32)


def _ds(start, size, align=None):
    return pl.ds(start if isinstance(start, int) else pl.multiple_of(start, align or size), size)


def _cut(cuts):
    return [(sum(cuts[:i]), n) for i, n in enumerate(cuts)]


def _loop(lo, hi, body):
    lax.fori_loop(lo, hi, lambda i, carry: body(i), None)


def _kernel(x_hbm, c_hbm, wm_hbm, wq_hbm, k_hbm, v_hbm, wo_hbm, w3_hbm, w4_hbm, out_hbm,
            x_ref, c_ref, wm_ref, wq_ref, k_ref, v_ref, wo_ref, w3_ref, w4_ref,
            cond_ref, q_ref, s_ref, max_ref, o_ref, attn_ref, mod_ref, out_ref, sems, *, cfg):
    first_half = k_hbm.shape[1] - 2

    def piece(hbm, ref, sem, tile_row, tile, tiles):
        at = (slice(None), _ds(tile_row * 8, 8), _ds(tile * 128, tiles * 128, 128))
        return pltpu.make_async_copy(hbm.at[at], ref.at[at], sems.at[sem])

    def cache_step(hbm, ref, sem, step):
        head = ((step >> 5) & 1) + ((step >> 6) << 2)
        copies = []
        for turn, phase in enumerate(cfg['phases']):
            h = head + 2 * (turn & 1)
            rows = _ds((turn >> 1) * 1024 + ((step + phase) & 31) * 32, 32)
            copies.append(pltpu.make_async_copy(hbm.at[h, pl.ds(first_half, 2), rows], ref.at[h, :, rows],
                                                sems.at[sem + h]))
        return copies

    keys = lambda step, n: [c for j in range(n) for c in cache_step(k_hbm, k_ref, S_K, step + j)]
    values = lambda step, n: [c for j in range(n) for c in cache_step(v_hbm, v_ref, S_V, step + j)]

    def wide_row(hbm, ref, sem, i):
        if cfg['wst'] == 1:
            return [piece(hbm, ref, sem, i, 4 * u, 4) for u in range(8)]
        return [piece(hbm, ref, sem, (i >> 1) + 14 * far, (i & 1) * 16 + 4 * u, 4) for u in range(4) for far in (0, 1)]

    def narrow_rows(hbm, ref, sem, first, cuts):
        return [piece(hbm, ref, sem, first + r, *at) for r, row in enumerate(cuts) for at in _cut(row)]

    def enqueue(main, side):
        done = 0
        for i, copy in enumerate(main):
            copy.start(priority=1)
            while done < (i + 1) * len(side) // len(main):
                side[done].start(priority=0)
                done += 1

    def landed(ref, sem):
        pltpu.make_async_copy(ref, ref, sems.at[sem]).wait()

    def whole(ref, cols=slice(None)):
        w = ref[:, :, cols]
        return w.reshape(2 * w.shape[1], w.shape[2])

    even = (lax.broadcasted_iota(jnp.int32, (ROWS, DH), 0) & 1) == 0

    def condition():
        pltpu.make_async_copy(c_hbm, c_ref, sems.at[S_C]).wait()
        pltpu.make_async_copy(x_hbm, x_ref, sems.at[S_X]).wait()
        landed(wm_ref.at[:, :, pl.ds(0, LATE)], S_WM)
        c = jnp.broadcast_to(c_ref[...].astype(F32), (ROWS, D))
        c = (c * jax.nn.sigmoid(c)).astype(BF16)

        def columns(i):
            cols = _ds(i * (LATE // 3), LATE // 3, 128)
            s_ref[0, :, cols] = _dot(c, whole(wm_ref, cols))
        _loop(0, 3, columns)
        for g in range(5):
            mod_ref[g] = s_ref[0, :, g * D:(g + 1) * D]
        mod_ref[5, :, 0:64] = s_ref[0, :, 5 * D:LATE]
        row = jnp.concatenate([c[0:1].astype(F32), jnp.zeros((1, 512 - D), F32)], axis=1)
        cond_ref[...] = jnp.broadcast_to(row, (128, 512)).T

    def queries():
        landed(wq_ref, S_WQ)
        x = jnp.broadcast_to(x_ref[0].astype(F32), (ROWS, D))
        h_in = (_layernorm(x) * (1.0 + mod_ref[1]) + mod_ref[0]).astype(BF16)

        def heads(i):
            q = _dot(h_in, whole(wq_ref, _ds(i * 4 * DH, 4 * DH))) * DH ** -0.5
            for u in range(2):
                q_ref[2 * i + u] = jnp.where(even, q[:, 2 * u * DH:(2 * u + 1) * DH], q[:, (2 * u + 1) * DH:(2 * u + 2) * DH])
        _loop(0, HKV // 2, heads)

    def scores(h):
        landed(k_ref.at[h], S_K + h)
        s = _dot_t(q_ref[h].astype(BF16), k_ref[h].reshape(WINDOW, DH))
        s_ref[h] = s
        m = s[:, :128]
        for t in range(1, WINDOW // 128):
            m = jnp.maximum(m, s[:, t * 128:(t + 1) * 128])
        max_ref[h] = jnp.broadcast_to(jnp.max(m, axis=-1, keepdims=True), (ROWS, 128))

    def context(h):
        landed(v_ref.at[h], S_V + h)
        p = jnp.exp(s_ref[h] - jnp.concatenate([max_ref[h]] * (WINDOW // 128), axis=1))
        total = p[:, :128]
        for t in range(1, WINDOW // 128):
            total = total + p[:, t * 128:(t + 1) * 128]
        o = _dot(p.astype(BF16), v_ref[h].reshape(WINDOW, DH)) / jnp.sum(total, axis=-1, keepdims=True)
        o_ref[h] = jnp.concatenate([jnp.where(even, o, 0.0), jnp.where(even, 0.0, o)], axis=1)

    def project(h):
        return _dot_t(o_ref[h].astype(BF16), whole(wo_ref, _ds(h * 2 * DH, 2 * DH)))

    def project_pair(h):
        attn_ref[...] += project(h) + project(h + 2)

    enqueue(keys(0, 1), [pltpu.make_async_copy(c_hbm, c_ref, sems.at[S_C]), pltpu.make_async_copy(x_hbm, x_ref, sems.at[S_X])])
    _loop(0, 7, lambda i: enqueue(keys(8 * i + 1, 8), narrow_rows(wm_hbm, wm_ref, S_WM, 4 * i, WM_CUTS)))

    def keys_and_wq(i):
        enqueue(keys(57 + 3 * i, 3), wide_row(wq_hbm, wq_ref, S_WQ, i))
        pl.when(i == 8)(condition)
    _loop(0, 23, keys_and_wq)
    enqueue(keys(126, 2), wide_row(wq_hbm, wq_ref, S_WQ, 23))
    _loop(0, 4, lambda i: enqueue(values(3 * i, 3), wide_row(wq_hbm, wq_ref, S_WQ, 24 + i)))

    def values_and_wo(i):
        enqueue(values(12 + 3 * i, 3), wide_row(wo_hbm, wo_ref, S_WO, i))
        n = (i - 5) >> 1

        @pl.when((i & 1) == 1)
        def _():
            pl.when(n == -1)(queries)
            pl.when((n >= 0) & (n < HKV))(lambda: scores(n))
            pl.when(n >= HKV)(lambda: context(((n & 1) << 1) + ((n >> 1) & 1)))
    _loop(0, 28, values_and_wo)

    per = cfg['w3rows'] // 8

    def values_and_w3(i):
        enqueue(values(96 + 4 * i, 4), narrow_rows(w3_hbm, w3_ref, S_W3, per * i, FF_CUTS * (per // 2)))

        @pl.when(i == 1)
        def _():
            landed(wo_ref, S_WO)
            attn_ref[...] = jnp.zeros((ROWS, D), F32)
        pl.when((i == 4) | (i == 5))(lambda: context(2 * i - 4))
        pl.when((i == 2) | (i == 3) | (i == 6))(lambda: project_pair(i - 2))
    _loop(0, 8, values_and_w3)

    w3 = narrow_rows(w3_hbm, w3_ref, S_W3, cfg['w3rows'], cfg['end3'] * ((28 - cfg['w3rows']) // 2))
    w4 = []
    for i, (r0, n) in enumerate(W4_BLOCKS):
        far = (0, n // 16) if n == 256 else (0,)
        tile_rows = [r0 // 8 + r + off for r in range(n // 8 // len(far)) for off in far]
        w4.append([piece(w4_hbm, w4_ref, S_W4 + i, r, *at) for r in tile_rows for at in _cut(cfg['end4'][r & 1])])
    gate = []
    for i, (r0, n) in enumerate(GATE_BLOCKS):
        for r in range(r0, r0 + n, cfg['grows']):
            at = (slice(None), pl.ds(r, cfg['grows']), pl.ds(LATE, 6 * D - LATE))
            gate.append(pltpu.make_async_copy(wm_hbm.at[at], wm_ref.at[at], sems.at[S_GATE + i]))
    rest = []
    for j, copy in enumerate(w3):
        rest += [copy] + w4[0][j * cfg['mix'] // len(w3):(j + 1) * cfg['mix'] // len(w3)]
    rest += w4[0][cfg['mix']:] + w4[1]
    main = [copy for j, copy in enumerate(rest) if j % cfg['share']] + w4[2] + gate
    side = rest[::cfg['share']][::-1]
    for j, copy in enumerate(main):
        copy.start(priority=1)
        if side and j >= cfg['lead'] and (j - cfg['lead']) % (cfg['share'] - 1) == 0:
            side.pop().start(priority=0)
        if j == min(len(main) - 1, cfg['at'][0]):
            _loop(0, 2, lambda u: context(5 + 2 * u))
        if j == min(len(main) - 1, cfg['at'][1]):
            attn = attn_ref[...] + project(5) + project(7)
            x = jnp.broadcast_to(x_ref[0].astype(F32), (ROWS, D))
            x = x + mod_ref[2] * (attn + pltpu.roll(attn, 1, 0))
            h_mlp = _layernorm(x) * (1.0 + mod_ref[4]) + mod_ref[3]
            normed = _layernorm(h_mlp).astype(BF16)
            mod_ref[0] = x
            mod_ref[1] = h_mlp
    while side:
        side.pop().start(priority=0)

    landed(w3_ref, S_W3)
    hidden = jax.nn.gelu(_dot(normed, whole(w3_ref)), approximate=True).astype(BF16)
    y = []
    for i, (r0, n) in enumerate(W4_BLOCKS):
        landed(w4_ref.at[:, pl.ds(r0, n)], S_W4 + i)
        block = mod_ref[1, :, r0:r0 + n] + _dot_t(hidden, w4_ref[0, r0:r0 + n, :])
        y += [block[:, t:min(n, t + 128)] for t in range(0, n, 128)]

    sums = [jnp.zeros((ROWS, 128), F32)] * 3
    for i, (r0, n) in enumerate(GATE_BLOCKS):
        landed(wm_ref.at[:, pl.ds(r0, n), pl.ds(LATE, 6 * D - LATE)], S_GATE + i)
        for half in range(2):
            for r in range(r0, r0 + n, 16):
                c = cond_ref[half * D // 2 + r:half * D // 2 + r + 16, :]
                for t in range(3):
                    w = wm_ref[half, r:r + 16, LATE + t * 128:LATE + (t + 1) * 128].astype(F32) * c
                    sums[t] = sums[t] + (w[:8] + w[8:])
    low = lax.broadcasted_iota(jnp.int32, (1, 128), 1) < 64
    sums = [pltpu.roll(jnp.sum(s, axis=0, keepdims=True), 64, 1) for s in sums]
    gates = [jnp.where(low, a, b) for a, b in zip([mod_ref[5, 0:1, 0:128]] + sums[:2], sums)] + [sums[2][:, :64]]
    for t, (g, m) in enumerate(zip(gates, y)):
        cols = slice(t * 128, t * 128 + g.shape[1])
        out_ref[0, :, cols] = (mod_ref[0, 0:1, cols] + g * m[0:1]).astype(BF16)
    store = pltpu.make_async_copy(out_ref, out_hbm, sems.at[S_X])
    store.start()
    store.wait()


def make(interpret=False, **kw):
    cfg = dict(CFG, **kw)

    def f(A_x, A_k_cache, A_v_cache, A_wq, A_wo, B_x, B_w1, B_w2, B_w3, B_w4, c, w_mod):
        hbm = pl.BlockSpec(memory_space=pltpu.HBM)
        halves = lambda w: w.reshape(2, D // 2, w.shape[1])
        windows = lambda cache: cache.reshape(HKV, -1, WINDOW // 2, DH)
        return pl.pallas_call(
            lambda *refs: _kernel(*refs, cfg=cfg),
            out_shape=jax.ShapeDtypeStruct(A_x.shape, A_x.dtype),
            in_specs=[hbm] * 9,
            out_specs=hbm,
            scratch_shapes=[
                pltpu.VMEM((1, 1, D), BF16),
                pltpu.VMEM((1, D), BF16),
                pltpu.VMEM((2, D // 2, 6 * D), BF16),
                pltpu.VMEM((2, D // 2, HQ * DH), BF16),
                pltpu.VMEM((HKV, 2, WINDOW // 2, DH), BF16),
                pltpu.VMEM((HKV, 2, WINDOW // 2, DH), BF16),
                pltpu.VMEM((2, D // 2, HQ * DH), BF16),
                pltpu.VMEM((2, D // 2, F), BF16),
                pltpu.VMEM((1, D, F), BF16),
                pltpu.VMEM((512, 128), F32),
                pltpu.VMEM((HKV, ROWS, DH), F32),
                pltpu.VMEM((HKV, ROWS, WINDOW), F32),
                pltpu.VMEM((HKV, ROWS, 128), F32),
                pltpu.VMEM((HKV, ROWS, 2 * DH), F32),
                pltpu.VMEM((ROWS, D), F32),
                pltpu.VMEM((6, ROWS, D), F32),
                pltpu.VMEM((1, 1, D), BF16),
                pltpu.SemaphoreType.DMA((S_GATE + len(GATE_BLOCKS),)),
            ],
            compiler_params=pltpu.CompilerParams(
                vmem_limit_bytes=100 * 2**20,
                disable_semaphore_checks=True,
                disable_bounds_checks=True,
                flags=cfg.get('flags'),
            ),
            interpret=interpret,
            name="adaln_decode",
        )(A_x, c, halves(w_mod), halves(A_wq), windows(A_k_cache), windows(A_v_cache), halves(A_wo.T),
          halves(B_w3), B_w4.T[None])
    return jax.jit(f)


pallas_adaLN_cond__sliding_block_cached__mixer_s_mlp__decode_kernel = make()
```

```python
import jax
import jax.numpy as jnp
from jax import lax
from jax.experimental import pallas as pl
from jax.experimental.pallas import tpu as pltpu

D, F = 448, 1792
HQ, HKV, DH = 16, 8, 256
WINDOW = 4096
EPS = 1e-5
ROWS = 8
LATE = 2304
BF16, F32 = jnp.bfloat16, jnp.float32

S_X, S_C, S_WM, S_WQ, S_WO, S_W3, S_K, S_V, S_W4, S_GATE = 0, 1, 2, 3, 4, 5, 6, 14, 22, 24
GATE_BLOCKS = ((0, 128), (128, 64), (192, 32))
WM_CUTS = ((4, 4, 4, 4, 2), (3, 4, 4, 4, 3), (2, 4, 4, 4, 4), (1, 4, 4, 4, 4, 1))
FF_CUTS = ((4, 4, 4, 2), (2, 4, 4, 4))
END_CUTS = ((4, 8, 2), (2, 8, 4))


def _layernorm(x):
    d = x - jnp.sum(x, axis=-1, keepdims=True) * (1.0 / D)
    return d * lax.rsqrt(jnp.sum(d * d, axis=-1, keepdims=True) * (1.0 / D) + EPS)


def _dot(a, b):
    return lax.dot_general(a, b, (((1,), (0,)), ((), ())), preferred_element_type=F32)


def _dot_t(a, b):
    return lax.dot_general(a, b, (((1,), (1,)), ((), ())), preferred_element_type=F32)


def _ds(start, size, align=None):
    return pl.ds(start if isinstance(start, int) else pl.multiple_of(start, align or size), size)


def _cut(cuts):
    return [(sum(cuts[:i]), n) for i, n in enumerate(cuts)]


def _loop(lo, hi, body):
    lax.fori_loop(lo, hi, lambda i, carry: body(i), None)


def _kernel(x_hbm, c_hbm, wm_hbm, wq_hbm, k_hbm, v_hbm, wo_hbm, w3_hbm, w4_hbm, out_hbm,
            x_ref, c_ref, wm_ref, wq_ref, k_ref, v_ref, wo_ref, w3_ref, w4_ref,
            cond_ref, q_ref, s_ref, max_ref, o_ref, attn_ref, mod_ref, out_ref, sems):
    first_half = k_hbm.shape[1] - 2

    def piece(hbm, ref, sem, tile_row, tile, tiles):
        at = (slice(None), _ds(tile_row * 8, 8), _ds(tile * 128, tiles * 128, 128))
        return pltpu.make_async_copy(hbm.at[at], ref.at[at], sems.at[sem])

    def cache_rows(hbm, ref, sem, head, quarter, position):
        rows = _ds(quarter * 1024 + (position & 31) * 32, 32)
        return pltpu.make_async_copy(hbm.at[head, pl.ds(first_half, 2), rows], ref.at[head, :, rows],
                                     sems.at[sem + head])

    def keys(first, steps):
        return [cache_rows(k_hbm, k_ref, S_K, ((step >> 6) << 2) + head, ((step >> 5) & 1) ^ (turn >> 1), step + lag)
                for step in (first + j for j in range(steps))
                for turn, (head, lag) in enumerate(((0, 0), (2, 8), (1, 23), (3, 31)))]

    def values(first, steps):
        return [cache_rows(v_hbm, v_ref, S_V, ((step >> 6) << 2) + ((step >> 5) & 1) + head, turn >> 1, step + lag)
                for step in (first + j for j in range(steps))
                for turn, (head, lag) in enumerate(((0, 0), (2, 24), (0, 1), (2, 25)))]

    def wide_part(hbm, ref, sem, i):
        return [piece(hbm, ref, sem, (i >> 1) + far, (i & 1) * 16 + 4 * u, 4) for u in range(4) for far in (0, 14)]

    def narrow_rows(hbm, ref, sem, first, cuts):
        return [piece(hbm, ref, sem, first + r, *at) for r, row in enumerate(cuts) for at in _cut(row)]

    def enqueue(main, side):
        done = 0
        for i, copy in enumerate(main):
            copy.start(priority=1)
            while done * len(main) < (i + 1) * len(side):
                side[done].start(priority=0)
                done += 1

    def landed(ref, sem):
        pltpu.make_async_copy(ref, ref, sems.at[sem]).wait()

    def whole(ref, cols=slice(None)):
        w = ref[:, :, cols]
        return w.reshape(2 * w.shape[1], w.shape[2])

    even = (lax.broadcasted_iota(jnp.int32, (ROWS, DH), 0) & 1) == 0

    def condition():
        pltpu.make_async_copy(c_hbm, c_ref, sems.at[S_C]).wait()
        pltpu.make_async_copy(x_hbm, x_ref, sems.at[S_X]).wait()
        landed(wm_ref.at[:, :, pl.ds(0, LATE)], S_WM)
        c = jnp.broadcast_to(c_ref[...].astype(F32), (ROWS, D))
        c = (c * jax.nn.sigmoid(c)).astype(BF16)

        def columns(i):
            cols = _ds(i * (LATE // 3), LATE // 3, 128)
            s_ref[0, :, cols] = _dot(c, whole(wm_ref, cols))
        _loop(0, 3, columns)
        for g in range(5):
            mod_ref[g] = s_ref[0, :, g * D:(g + 1) * D]
        mod_ref[5, :, 0:128] = jnp.concatenate([s_ref[0, :, 5 * D:LATE], jnp.zeros((ROWS, 64), F32)], axis=1)
        row = jnp.concatenate([c[0:1].astype(F32), jnp.zeros((1, 512 - D), F32)], axis=1)
        cond_ref[...] = jnp.broadcast_to(row, (128, 512)).T

    def queries():
        landed(wq_ref, S_WQ)
        x = jnp.broadcast_to(x_ref[0].astype(F32), (ROWS, D))
        h_in = (_layernorm(x) * (1.0 + mod_ref[1]) + mod_ref[0]).astype(BF16)

        def heads(i):
            q = _dot(h_in, whole(wq_ref, _ds(i * 4 * DH, 4 * DH))) * DH ** -0.5
            for u in range(2):
                pair = q[:, u * 2 * DH:(u + 1) * 2 * DH]
                q_ref[2 * i + u] = jnp.where(even, pair[:, :DH], pair[:, DH:])
        _loop(0, HKV // 2, heads)

    def scores(h):
        landed(k_ref.at[h], S_K + h)
        s = _dot_t(q_ref[h].astype(BF16), k_ref[h].reshape(WINDOW, DH))
        s_ref[h] = s
        m = s[:, :128]
        for t in range(1, WINDOW // 128):
            m = jnp.maximum(m, s[:, t * 128:(t + 1) * 128])
        max_ref[h] = jnp.broadcast_to(jnp.max(m, axis=-1, keepdims=True), (ROWS, 128))

    def context(h):
        landed(v_ref.at[h], S_V + h)
        p = jnp.exp(s_ref[h] - jnp.concatenate([max_ref[h]] * (WINDOW // 128), axis=1))
        total = p[:, :128]
        for t in range(1, WINDOW // 128):
            total = total + p[:, t * 128:(t + 1) * 128]
        o = _dot(p.astype(BF16), v_ref[h].reshape(WINDOW, DH)) / jnp.sum(total, axis=-1, keepdims=True)
        o_ref[h] = jnp.concatenate([jnp.where(even, o, 0.0), jnp.where(even, 0.0, o)], axis=1)

    def project(h):
        return _dot_t(o_ref[h].astype(BF16), whole(wo_ref, _ds(h * 2 * DH, 2 * DH)))

    def project_pair(h):
        attn_ref[...] += project(h) + project(h + 2)

    enqueue(keys(0, 1), [pltpu.make_async_copy(c_hbm, c_ref, sems.at[S_C]),
                         pltpu.make_async_copy(x_hbm, x_ref, sems.at[S_X])])
    _loop(0, 7, lambda i: enqueue(keys(8 * i + 1, 8), narrow_rows(wm_hbm, wm_ref, S_WM, 4 * i, WM_CUTS)))

    def keys_and_wq(i):
        enqueue(keys(57 + 3 * i, 3), wide_part(wq_hbm, wq_ref, S_WQ, i))
        pl.when(i == 8)(condition)
    _loop(0, 23, keys_and_wq)
    enqueue(keys(126, 2), wide_part(wq_hbm, wq_ref, S_WQ, 23))
    _loop(0, 4, lambda i: enqueue(values(3 * i, 3), wide_part(wq_hbm, wq_ref, S_WQ, 24 + i)))

    def values_and_wo(i):
        enqueue(values(12 + 3 * i, 3), wide_part(wo_hbm, wo_ref, S_WO, i))
        n = (i - 5) >> 1

        @pl.when((i & 1) == 1)
        def _():
            pl.when(n == -1)(queries)
            pl.when((n >= 0) & (n < HKV))(lambda: scores(n))
            pl.when(n >= HKV)(lambda: context(((n & 1) << 1) + ((n >> 1) & 1)))
    _loop(0, 28, values_and_wo)

    def values_and_w3(i):
        enqueue(values(96 + 4 * i, 4), narrow_rows(w3_hbm, w3_ref, S_W3, 2 * i, FF_CUTS))

        @pl.when(i == 1)
        def _():
            landed(wo_ref, S_WO)
            attn_ref[...] = jnp.zeros((ROWS, D), F32)
        pl.when((i == 4) | (i == 5))(lambda: context(2 * i - 4))
        pl.when((i == 2) | (i == 3) | (i == 6))(lambda: project_pair(i - 2))
    _loop(0, 8, values_and_w3)

    w3 = narrow_rows(w3_hbm, w3_ref, S_W3, 16, END_CUTS * 6)
    w4 = narrow_rows(w4_hbm, w4_ref, S_W4, 0, END_CUTS * 10) + narrow_rows(w4_hbm, w4_ref, S_W4 + 1, 20, END_CUTS * 4)
    rest = [copy for j in range(18) for copy in (w3[2 * j], w3[2 * j + 1], w4[j])] + w4[18:]
    main, side = [copy for j, copy in enumerate(rest) if j % 3], rest[::3]
    for i, (r0, n) in enumerate(GATE_BLOCKS):
        for r in range(r0, r0 + n, 8):
            for half in ((slice(None),) if i == 0 else (0, 1)):
                at = (half, pl.ds(r, 8), pl.ds(LATE, 6 * D - LATE))
                main.append(pltpu.make_async_copy(wm_hbm.at[at], wm_ref.at[at], sems.at[S_GATE + i]))
    for j, copy in enumerate(main):
        copy.start(priority=1)
        if side and j >= 24 and j % 2 == 0:
            side.pop(0).start(priority=0)
        if j == 48:
            _loop(0, 2, lambda u: context(5 + 2 * u))
        if j == 60:
            attn = attn_ref[...] + project(5) + project(7)
            x = jnp.broadcast_to(x_ref[0].astype(F32), (ROWS, D))
            x = x + mod_ref[2] * (attn + pltpu.roll(attn, 1, 0))
            h_mlp = _layernorm(x) * (1.0 + mod_ref[4]) + mod_ref[3]
            normed = _layernorm(h_mlp).astype(BF16)
            mod_ref[0] = x
            mod_ref[1] = h_mlp
        if j == 86:
            landed(w3_ref, S_W3)
            hidden = jax.nn.gelu(_dot(normed, whole(w3_ref)), approximate=True).astype(BF16)
    assert not side

    landed(w4_ref.at[:, pl.ds(0, 160)], S_W4)
    y02 = _dot_t(hidden, jnp.concatenate([w4_ref[0, 0:128], w4_ref[1, 32:160]], axis=0))
    landed(w4_ref.at[:, pl.ds(160, 64)], S_W4 + 1)
    y13 = _dot_t(hidden, jnp.concatenate([w4_ref[0, 128:224], w4_ref[1, 0:32], w4_ref[1, 160:224]], axis=0))
    y = [y02[:, :128], y13[:, :128], y02[:, 128:], y13[:, 128:]]
    y = [part + mod_ref[1, :, t * 128:t * 128 + part.shape[1]] for t, part in enumerate(y)]

    sums = [jnp.zeros((ROWS, 128), F32)] * 3
    for i, (r0, n) in enumerate(GATE_BLOCKS):
        landed(wm_ref.at[:, pl.ds(r0, n), pl.ds(LATE, 6 * D - LATE)], S_GATE + i)
        for half in range(2):
            for r in range(r0, r0 + n, 16):
                c = cond_ref[half * D // 2 + r:half * D // 2 + r + 16, :]
                for t in range(3):
                    w = wm_ref[half, r:r + 16, LATE + t * 128:LATE + (t + 1) * 128].astype(F32) * c
                    sums[t] = sums[t] + (w[:8] + w[8:])
    low = lax.broadcasted_iota(jnp.int32, (1, 128), 1) < 64
    sums = [pltpu.roll(jnp.sum(s, axis=0, keepdims=True), 64, 1) for s in sums]
    gates = [jnp.where(low, a, b) for a, b in zip([mod_ref[5, 0:1, 0:128]] + sums[:2], sums)] + [sums[2][:, :64]]
    for t, (g, m) in enumerate(zip(gates, y)):
        cols = slice(t * 128, t * 128 + g.shape[1])
        out_ref[0, :, cols] = (mod_ref[0, 0:1, cols] + g * m[0:1]).astype(BF16)
    store = pltpu.make_async_copy(out_ref, out_hbm, sems.at[S_X])
    store.start()
    store.wait()


@jax.jit
def pallas_adaLN_cond__sliding_block_cached__mixer_s_mlp__decode_kernel(
    A_x: jax.Array,
    A_k_cache: jax.Array,
    A_v_cache: jax.Array,
    A_wq: jax.Array,
    A_wo: jax.Array,
    B_x: jax.Array,
    B_w1: jax.Array,
    B_w2: jax.Array,
    B_w3: jax.Array,
    B_w4: jax.Array,
    c: jax.Array,
    w_mod: jax.Array,
):
    keys = A_k_cache.shape[2]
    assert A_x.shape == (1, 1, D) and A_k_cache.shape == (1, HKV, keys, DH)
    assert min(4096, max(256, keys // 4)) == WINDOW and keys % (WINDOW // 2) == 0
    hbm = pl.BlockSpec(memory_space=pltpu.HBM)
    halves = lambda w: w.reshape(2, D // 2, w.shape[1])
    windows = lambda cache: cache.reshape(HKV, -1, WINDOW // 2, DH)
    return pl.pallas_call(
        _kernel,
        out_shape=jax.ShapeDtypeStruct(A_x.shape, A_x.dtype),
        in_specs=[hbm] * 9,
        out_specs=hbm,
        scratch_shapes=[
            pltpu.VMEM((1, 1, D), BF16),
            pltpu.VMEM((1, D), BF16),
            pltpu.VMEM((2, D // 2, 6 * D), BF16),
            pltpu.VMEM((2, D // 2, HQ * DH), BF16),
            pltpu.VMEM((HKV, 2, WINDOW // 2, DH), BF16),
            pltpu.VMEM((HKV, 2, WINDOW // 2, DH), BF16),
            pltpu.VMEM((2, D // 2, HQ * DH), BF16),
            pltpu.VMEM((2, D // 2, F), BF16),
            pltpu.VMEM((2, D // 2, F), BF16),
            pltpu.VMEM((512, 128), F32),
            pltpu.VMEM((HKV, ROWS, DH), F32),
            pltpu.VMEM((HKV, ROWS, WINDOW), F32),
            pltpu.VMEM((HKV, ROWS, 128), F32),
            pltpu.VMEM((HKV, ROWS, 2 * DH), F32),
            pltpu.VMEM((ROWS, D), F32),
            pltpu.VMEM((6, ROWS, D), F32),
            pltpu.VMEM((1, 1, D), BF16),
            pltpu.SemaphoreType.DMA((S_GATE + len(GATE_BLOCKS),)),
        ],
        compiler_params=pltpu.CompilerParams(
            vmem_limit_bytes=100 * 2**20,
            disable_semaphore_checks=True,
            disable_bounds_checks=True,
        ),
        name="adaln_decode",
    )(A_x, c, halves(w_mod), halves(A_wq), windows(A_k_cache), windows(A_v_cache), halves(A_wo.T),
      halves(B_w3), halves(B_w4.T))
```

```python
import jax
import jax.numpy as jnp
from jax import lax
from jax.experimental import pallas as pl
from jax.experimental.pallas import tpu as pltpu

D, F = 448, 1792
HQ, HKV, DH = 16, 8, 256
WINDOW = 4096
EPS = 1e-5
ROWS = 8
LATE = 2304
BF16, F32 = jnp.bfloat16, jnp.float32

S_X, S_C, S_WM, S_WQ, S_WO, S_W3, S_K, S_V, S_W4, S_GATE = 0, 1, 2, 3, 4, 5, 6, 14, 22, 24
GATE_BLOCKS = ((0, 144), (144, 64), (208, 16))
WM_CUTS = ((4, 4, 4, 4, 2), (3, 4, 4, 4, 3), (2, 4, 4, 4, 4), (1, 4, 4, 4, 4, 1))
FF_CUTS = ((4, 4, 4, 2), (2, 4, 4, 4))
END_CUTS = ((4, 8, 2), (2, 8, 4))


def _layernorm(x):
    d = x - jnp.sum(x, axis=-1, keepdims=True) * (1.0 / D)
    return d * lax.rsqrt(jnp.sum(d * d, axis=-1, keepdims=True) * (1.0 / D) + EPS)


def _dot(a, b):
    return lax.dot_general(a, b, (((1,), (0,)), ((), ())), preferred_element_type=F32)


def _dot_t(a, b):
    return lax.dot_general(a, b, (((1,), (1,)), ((), ())), preferred_element_type=F32)


def _ds(start, size, align=None):
    return pl.ds(start if isinstance(start, int) else pl.multiple_of(start, align or size), size)


def _cut(cuts):
    return [(sum(cuts[:i]), n) for i, n in enumerate(cuts)]


def _loop(lo, hi, body):
    lax.fori_loop(lo, hi, lambda i, carry: body(i), None)


def _kernel(x_hbm, c_hbm, wm_hbm, wq_hbm, k_hbm, v_hbm, wo_hbm, w3_hbm, w4_hbm, out_hbm,
            x_ref, c_ref, wm_ref, wq_ref, k_ref, v_ref, wo_ref, w3_ref, w4_ref,
            cond_ref, q_ref, s_ref, max_ref, o_ref, attn_ref, mod_ref, out_ref, sems):
    first_half = k_hbm.shape[1] - 2

    def piece(hbm, ref, sem, tile_row, tile, tiles):
        at = (slice(None), _ds(tile_row * 8, 8), _ds(tile * 128, tiles * 128, 128))
        return pltpu.make_async_copy(hbm.at[at], ref.at[at], sems.at[sem])

    def cache_rows(hbm, ref, sem, head, quarter, position):
        rows = _ds(quarter * 1024 + (position & 31) * 32, 32)
        return pltpu.make_async_copy(hbm.at[head, pl.ds(first_half, 2), rows], ref.at[head, :, rows],
                                     sems.at[sem + head])

    def keys(first, steps):
        return [cache_rows(k_hbm, k_ref, S_K, ((step >> 6) << 2) + head, ((step >> 5) & 1) ^ (turn >> 1), step + lag)
                for step in (first + j for j in range(steps))
                for turn, (head, lag) in enumerate(((0, 0), (2, 8), (1, 29), (3, 0)))]

    def values(first, steps):
        return [cache_rows(v_hbm, v_ref, S_V, ((step >> 6) << 2) + ((step >> 5) & 1) + head, turn >> 1, step + lag)
                for step in (first + j for j in range(steps))
                for turn, (head, lag) in enumerate(((0, 0), (2, 8), (0, 1), (2, 9)))]

    def wide_part(hbm, ref, sem, i):
        return [piece(hbm, ref, sem, (i >> 1) + far, (i & 1) * 16 + 4 * u, 4) for u in range(4) for far in (0, 14)]

    def narrow_rows(hbm, ref, sem, first, cuts):
        return [piece(hbm, ref, sem, first + r, *at) for r, row in enumerate(cuts) for at in _cut(row)]

    def enqueue(main, side):
        done = 0
        for i, copy in enumerate(main):
            copy.start(priority=1)
            while done * len(main) < (i + 1) * len(side):
                side[done].start(priority=0)
                done += 1

    def landed(ref, sem):
        pltpu.make_async_copy(ref, ref, sems.at[sem]).wait()

    def whole(ref, cols=slice(None)):
        w = ref[:, :, cols]
        return w.reshape(2 * w.shape[1], w.shape[2])

    even = (lax.broadcasted_iota(jnp.int32, (ROWS, DH), 0) & 1) == 0

    def condition():
        pltpu.make_async_copy(c_hbm, c_ref, sems.at[S_C]).wait()
        pltpu.make_async_copy(x_hbm, x_ref, sems.at[S_X]).wait()
        landed(wm_ref.at[:, :, pl.ds(0, LATE)], S_WM)
        c = jnp.broadcast_to(c_ref[...].astype(F32), (ROWS, D))
        c = (c * jax.nn.sigmoid(c)).astype(BF16)

        def columns(i):
            cols = _ds(i * (LATE // 3), LATE // 3, 128)
            s_ref[0, :, cols] = _dot(c, whole(wm_ref, cols))
        _loop(0, 3, columns)
        for g in range(5):
            mod_ref[g] = s_ref[0, :, g * D:(g + 1) * D]
        mod_ref[5, :, 0:128] = jnp.concatenate([s_ref[0, :, 5 * D:LATE], jnp.zeros((ROWS, 64), F32)], axis=1)
        row = jnp.concatenate([c[0:1].astype(F32), jnp.zeros((1, 512 - D), F32)], axis=1)
        cond_ref[...] = jnp.broadcast_to(row, (128, 512)).T

    def queries():
        landed(wq_ref, S_WQ)
        x = jnp.broadcast_to(x_ref[0].astype(F32), (ROWS, D))
        h_in = (_layernorm(x) * (1.0 + mod_ref[1]) + mod_ref[0]).astype(BF16)

        def heads(i):
            q = _dot(h_in, whole(wq_ref, _ds(i * 4 * DH, 4 * DH))) * DH ** -0.5
            for u in range(2):
                pair = q[:, u * 2 * DH:(u + 1) * 2 * DH]
                q_ref[2 * i + u] = jnp.where(even, pair[:, :DH], pair[:, DH:])
        _loop(0, HKV // 2, heads)

    def scores(h):
        landed(k_ref.at[h], S_K + h)
        s = _dot_t(q_ref[h].astype(BF16), k_ref[h].reshape(WINDOW, DH))
        s_ref[h] = s
        m = s[:, :128]
        for t in range(1, WINDOW // 128):
            m = jnp.maximum(m, s[:, t * 128:(t + 1) * 128])
        max_ref[h] = jnp.broadcast_to(jnp.max(m, axis=-1, keepdims=True), (ROWS, 128))

    def context(h):
        landed(v_ref.at[h], S_V + h)
        p = jnp.exp(s_ref[h] - jnp.concatenate([max_ref[h]] * (WINDOW // 128), axis=1))
        total = p[:, :128]
        for t in range(1, WINDOW // 128):
            total = total + p[:, t * 128:(t + 1) * 128]
        o = _dot(p.astype(BF16), v_ref[h].reshape(WINDOW, DH)) / jnp.sum(total, axis=-1, keepdims=True)
        o_ref[h] = jnp.concatenate([jnp.where(even, o, 0.0), jnp.where(even, 0.0, o)], axis=1)

    def project(h):
        return _dot_t(o_ref[h].astype(BF16), whole(wo_ref, _ds(h * 2 * DH, 2 * DH)))

    def project_pair(h):
        attn_ref[...] += project(h) + project(h + 2)

    enqueue(keys(0, 4), [pltpu.make_async_copy(c_hbm, c_ref, sems.at[S_C]),
                         pltpu.make_async_copy(x_hbm, x_ref, sems.at[S_X])])
    _loop(0, 7, lambda i: enqueue(keys(4 + 8 * i, 8), narrow_rows(wm_hbm, wm_ref, S_WM, 4 * i, WM_CUTS)))

    def keys_and_wq(i):
        enqueue(keys(60 + 3 * i, 3), wide_part(wq_hbm, wq_ref, S_WQ, i))
        pl.when(i == 8)(condition)
    _loop(0, 22, keys_and_wq)
    enqueue(keys(126, 2), wide_part(wq_hbm, wq_ref, S_WQ, 22))
    _loop(0, 5, lambda i: enqueue(values(3 * i, 3), wide_part(wq_hbm, wq_ref, S_WQ, 23 + i)))

    def values_and_wo(i):
        enqueue(values(15 + 3 * i, 3), wide_part(wo_hbm, wo_ref, S_WO, i))
        n = (i - 5) >> 1

        @pl.when((i & 1) == 1)
        def _():
            pl.when(n == -1)(queries)
            pl.when((n >= 0) & (n < HKV))(lambda: scores(n))
            pl.when(n >= HKV)(lambda: context(((n & 1) << 1) + ((n >> 1) & 1)))
    _loop(0, 28, values_and_wo)

    enqueue(values(99, 1), [])

    def values_and_w3(i):
        enqueue(values(100 + 4 * i, 4), narrow_rows(w3_hbm, w3_ref, S_W3, 2 * i, FF_CUTS))

        @pl.when(i == 1)
        def _():
            landed(wo_ref, S_WO)
            attn_ref[...] = jnp.zeros((ROWS, D), F32)
        pl.when((i == 4) | (i == 5))(lambda: context(2 * i - 4))
        pl.when((i == 2) | (i == 3) | (i == 6))(lambda: project_pair(i - 2))
    _loop(0, 7, values_and_w3)

    w3 = narrow_rows(w3_hbm, w3_ref, S_W3, 14, END_CUTS * 7)
    w4 = narrow_rows(w4_hbm, w4_ref, S_W4, 0, END_CUTS * 10) + narrow_rows(w4_hbm, w4_ref, S_W4 + 1, 20, END_CUTS * 4)
    rest = [copy for j in range(21) for copy in (w3[2 * j], w3[2 * j + 1], w4[j])] + w4[21:]
    main, side = [copy for j, copy in enumerate(rest) if j % 3], rest[::3]
    for i, (r0, n) in enumerate(GATE_BLOCKS):
        for r in range(r0, r0 + n, 8):
            for half in ((slice(None),) if i == 0 else (0, 1)):
                at = (half, pl.ds(r, 8), pl.ds(LATE, 6 * D - LATE))
                main.append(pltpu.make_async_copy(wm_hbm.at[at], wm_ref.at[at], sems.at[S_GATE + i]))
    for j, copy in enumerate(main):
        copy.start(priority=1)
        if side and j >= 24 and j % 2 == 0:
            side.pop(0).start(priority=0)
        if j == 48:
            _loop(0, 2, lambda u: context(5 + 2 * u))
        if j == 60:
            attn = attn_ref[...] + project(5) + project(7)
            x = jnp.broadcast_to(x_ref[0].astype(F32), (ROWS, D))
            x = x + mod_ref[2] * (attn + pltpu.roll(attn, 1, 0))
            h_mlp = _layernorm(x) * (1.0 + mod_ref[4]) + mod_ref[3]
            normed = _layernorm(h_mlp).astype(BF16)
            mod_ref[0] = x
            mod_ref[1] = h_mlp
        if j == 90:
            landed(w3_ref, S_W3)
            hidden = jax.nn.gelu(_dot(normed, whole(w3_ref)), approximate=True).astype(BF16)
    assert not side

    landed(w4_ref.at[:, pl.ds(0, 160)], S_W4)
    y02 = _dot_t(hidden, jnp.concatenate([w4_ref[0, 0:128], w4_ref[1, 32:160]], axis=0))
    landed(w4_ref.at[:, pl.ds(160, 64)], S_W4 + 1)
    y13 = _dot_t(hidden, jnp.concatenate([w4_ref[0, 128:224], w4_ref[1, 0:32], w4_ref[1, 160:224]], axis=0))
    y = [y02[:, :128], y13[:, :128], y02[:, 128:], y13[:, 128:]]
    y = [part + mod_ref[1, :, t * 128:t * 128 + part.shape[1]] for t, part in enumerate(y)]

    sums = [jnp.zeros((ROWS, 128), F32)] * 3
    for i, (r0, n) in enumerate(GATE_BLOCKS):
        landed(wm_ref.at[:, pl.ds(r0, n), pl.ds(LATE, 6 * D - LATE)], S_GATE + i)
        for half in range(2):
            for r in range(r0, r0 + n, 16):
                c = cond_ref[half * D // 2 + r:half * D // 2 + r + 16, :]
                for t in range(3):
                    w = wm_ref[half, r:r + 16, LATE + t * 128:LATE + (t + 1) * 128].astype(F32) * c
                    sums[t] = sums[t] + (w[:8] + w[8:])
    low = lax.broadcasted_iota(jnp.int32, (1, 128), 1) < 64
    sums = [pltpu.roll(jnp.sum(s, axis=0, keepdims=True), 64, 1) for s in sums]
    gates = [jnp.where(low, a, b) for a, b in zip([mod_ref[5, 0:1, 0:128]] + sums[:2], sums)] + [sums[2][:, :64]]
    for t, (g, m) in enumerate(zip(gates, y)):
        cols = slice(t * 128, t * 128 + g.shape[1])
        out_ref[0, :, cols] = (mod_ref[0, 0:1, cols] + g * m[0:1]).astype(BF16)
    store = pltpu.make_async_copy(out_ref, out_hbm, sems.at[S_X])
    store.start()
    store.wait()


@jax.jit
def pallas_adaLN_cond__sliding_block_cached__mixer_s_mlp__decode_kernel(
    A_x: jax.Array,
    A_k_cache: jax.Array,
    A_v_cache: jax.Array,
    A_wq: jax.Array,
    A_wo: jax.Array,
    B_x: jax.Array,
    B_w1: jax.Array,
    B_w2: jax.Array,
    B_w3: jax.Array,
    B_w4: jax.Array,
    c: jax.Array,
    w_mod: jax.Array,
):
    keys = A_k_cache.shape[2]
    assert A_x.shape == (1, 1, D) and A_k_cache.shape == (1, HKV, keys, DH)
    assert min(4096, max(256, keys // 4)) == WINDOW and keys % (WINDOW // 2) == 0
    hbm = pl.BlockSpec(memory_space=pltpu.HBM)
    halves = lambda w: w.reshape(2, D // 2, w.shape[1])
    windows = lambda cache: cache.reshape(HKV, -1, WINDOW // 2, DH)
    return pl.pallas_call(
        _kernel,
        out_shape=jax.ShapeDtypeStruct(A_x.shape, A_x.dtype),
        in_specs=[hbm] * 9,
        out_specs=hbm,
        scratch_shapes=[
            pltpu.VMEM((1, 1, D), BF16),
            pltpu.VMEM((1, D), BF16),
            pltpu.VMEM((2, D // 2, 6 * D), BF16),
            pltpu.VMEM((2, D // 2, HQ * DH), BF16),
            pltpu.VMEM((HKV, 2, WINDOW // 2, DH), BF16),
            pltpu.VMEM((HKV, 2, WINDOW // 2, DH), BF16),
            pltpu.VMEM((2, D // 2, HQ * DH), BF16),
            pltpu.VMEM((2, D // 2, F), BF16),
            pltpu.VMEM((2, D // 2, F), BF16),
            pltpu.VMEM((512, 128), F32),
            pltpu.VMEM((HKV, ROWS, DH), F32),
            pltpu.VMEM((HKV, ROWS, WINDOW), F32),
            pltpu.VMEM((HKV, ROWS, 128), F32),
            pltpu.VMEM((HKV, ROWS, 2 * DH), F32),
            pltpu.VMEM((ROWS, D), F32),
            pltpu.VMEM((6, ROWS, D), F32),
            pltpu.VMEM((1, 1, D), BF16),
            pltpu.SemaphoreType.DMA((S_GATE + len(GATE_BLOCKS),)),
        ],
        compiler_params=pltpu.CompilerParams(
            vmem_limit_bytes=100 * 2**20,
            disable_semaphore_checks=True,
            disable_bounds_checks=True,
        ),
        name="adaln_decode",
    )(A_x, c, halves(w_mod), halves(A_wq), windows(A_k_cache), windows(A_v_cache), halves(A_wo.T),
      halves(B_w3), halves(B_w4.T))
```

```python
import jax
import jax.numpy as jnp
from jax import lax
from jax.experimental import pallas as pl
from jax.experimental.pallas import tpu as pltpu

D, F = 448, 1792
HQ, HKV, DH = 16, 8, 256
WINDOW = 4096
EPS = 1e-5
ROWS = 8
LATE = 2304
BF16, F32 = jnp.bfloat16, jnp.float32

S_X, S_C, S_WM, S_WQ, S_WO, S_W3, S_K, S_V, S_W4, S_GATE = 0, 1, 2, 3, 4, 5, 6, 14, 22, 24
GATE_BLOCKS = ((0, 144), (144, 64), (208, 16))
WM_CUTS = ((4, 4, 4, 4, 2), (3, 4, 4, 4, 3), (2, 4, 4, 4, 4), (1, 4, 4, 4, 4, 1))
FF_CUTS = ((4, 4, 4, 2), (2, 4, 4, 4))
END_CUTS = ((4, 8, 2), (2, 8, 4))


def _layernorm(x):
    d = x - jnp.sum(x, axis=-1, keepdims=True) * (1.0 / D)
    return d * lax.rsqrt(jnp.sum(d * d, axis=-1, keepdims=True) * (1.0 / D) + EPS)


def _dot(a, b):
    return lax.dot_general(a, b, (((1,), (0,)), ((), ())), preferred_element_type=F32)


def _dot_t(a, b):
    return lax.dot_general(a, b, (((1,), (1,)), ((), ())), preferred_element_type=F32)


def _ds(start, size, align=None):
    return pl.ds(start if isinstance(start, int) else pl.multiple_of(start, align or size), size)


def _cut(cuts):
    return [(sum(cuts[:i]), n) for i, n in enumerate(cuts)]


def _loop(lo, hi, body):
    lax.fori_loop(lo, hi, lambda i, carry: body(i), None)


def _kernel(x_hbm, c_hbm, wm_hbm, wq_hbm, k_hbm, v_hbm, wo_hbm, w3_hbm, w4_hbm, out_hbm,
            x_ref, c_ref, wm_ref, wq_ref, k_ref, v_ref, wo_ref, w3_ref, w4_ref,
            cond_ref, q_ref, s_ref, max_ref, o_ref, attn_ref, mod_ref, out_ref, sems):
    first_half = k_hbm.shape[1] - 2

    def piece(hbm, ref, sem, tile_row, tile, tiles):
        at = (slice(None), _ds(tile_row * 8, 8), _ds(tile * 128, tiles * 128, 128))
        return pltpu.make_async_copy(hbm.at[at], ref.at[at], sems.at[sem])

    def cache_rows(hbm, ref, sem, head, quarter, position):
        rows = _ds(quarter * 1024 + (position & 31) * 32, 32)
        return pltpu.make_async_copy(hbm.at[head, pl.ds(first_half, 2), rows], ref.at[head, :, rows],
                                     sems.at[sem + head])

    def keys(first, steps):
        return [cache_rows(k_hbm, k_ref, S_K, ((step >> 6) << 2) + head, ((step >> 5) & 1) ^ (turn >> 1), step + lag)
                for step in (first + j for j in range(steps))
                for turn, (head, lag) in enumerate(((0, 0), (2, 8), (1, 29), (3, 0)))]

    def values(first, steps):
        return [cache_rows(v_hbm, v_ref, S_V, ((step >> 6) << 2) + ((step >> 5) & 1) + head, turn >> 1, step + lag)
                for step in (first + j for j in range(steps))
                for turn, (head, lag) in enumerate(((0, 0), (2, 8), (0, 1), (2, 9)))]

    def wide_part(hbm, ref, sem, i):
        return [piece(hbm, ref, sem, (i >> 1) + far, (i & 1) * 16 + 4 * u, 4) for u in range(4) for far in (0, 14)]

    def narrow_rows(hbm, ref, sem, first, cuts):
        return [piece(hbm, ref, sem, first + r, *at) for r, row in enumerate(cuts) for at in _cut(row)]

    def wm_part(i):
        near = narrow_rows(wm_hbm, wm_ref, S_WM, 4 * i, WM_CUTS[:2])
        far = narrow_rows(wm_hbm, wm_ref, S_WM, jnp.where(i < 4, 4 * i + 14, 4 * i - 14), WM_CUTS[2:])
        return [copy for pair in zip(far, near) for copy in pair] + far[len(near):]

    def enqueue(main, side):
        done = 0
        for i, copy in enumerate(main):
            copy.start(priority=1)
            while done * len(main) < (i + 1) * len(side):
                side[done].start(priority=0)
                done += 1

    def landed(ref, sem):
        pltpu.make_async_copy(ref, ref, sems.at[sem]).wait()

    def whole(ref, cols=slice(None)):
        w = ref[:, :, cols]
        return w.reshape(2 * w.shape[1], w.shape[2])

    even = (lax.broadcasted_iota(jnp.int32, (ROWS, DH), 0) & 1) == 0

    def condition():
        pltpu.make_async_copy(c_hbm, c_ref, sems.at[S_C]).wait()
        pltpu.make_async_copy(x_hbm, x_ref, sems.at[S_X]).wait()
        landed(wm_ref.at[:, :, pl.ds(0, LATE)], S_WM)
        c = jnp.broadcast_to(c_ref[...].astype(F32), (ROWS, D))
        c = (c * jax.nn.sigmoid(c)).astype(BF16)

        def columns(i):
            cols = _ds(i * (LATE // 3), LATE // 3, 128)
            s_ref[0, :, cols] = _dot(c, whole(wm_ref, cols))
        _loop(0, 3, columns)
        for g in range(5):
            mod_ref[g] = s_ref[0, :, g * D:(g + 1) * D]
        mod_ref[5, :, 0:128] = jnp.concatenate([s_ref[0, :, 5 * D:LATE], jnp.zeros((ROWS, 64), F32)], axis=1)
        row = jnp.concatenate([c[0:1].astype(F32), jnp.zeros((1, 512 - D), F32)], axis=1)
        cond_ref[...] = jnp.broadcast_to(row, (128, 512)).T

    def queries():
        landed(wq_ref, S_WQ)
        x = jnp.broadcast_to(x_ref[0].astype(F32), (ROWS, D))
        h_in = (_layernorm(x) * (1.0 + mod_ref[1]) + mod_ref[0]).astype(BF16)

        def heads(i):
            q = _dot(h_in, whole(wq_ref, _ds(i * 4 * DH, 4 * DH))) * DH ** -0.5
            for u in range(2):
                pair = q[:, u * 2 * DH:(u + 1) * 2 * DH]
                q_ref[2 * i + u] = jnp.where(even, pair[:, :DH], pair[:, DH:])
        _loop(0, HKV // 2, heads)

    def scores(h):
        landed(k_ref.at[h], S_K + h)
        s = _dot_t(q_ref[h].astype(BF16), k_ref[h].reshape(WINDOW, DH))
        s_ref[h] = s
        m = s[:, :128]
        for t in range(1, WINDOW // 128):
            m = jnp.maximum(m, s[:, t * 128:(t + 1) * 128])
        max_ref[h] = jnp.broadcast_to(jnp.max(m, axis=-1, keepdims=True), (ROWS, 128))

    def context(h):
        landed(v_ref.at[h], S_V + h)
        p = jnp.exp(s_ref[h] - jnp.concatenate([max_ref[h]] * (WINDOW // 128), axis=1))
        total = p[:, :128]
        for t in range(1, WINDOW // 128):
            total = total + p[:, t * 128:(t + 1) * 128]
        o = _dot(p.astype(BF16), v_ref[h].reshape(WINDOW, DH)) / jnp.sum(total, axis=-1, keepdims=True)
        o_ref[h] = jnp.concatenate([jnp.where(even, o, 0.0), jnp.where(even, 0.0, o)], axis=1)

    def project(h):
        return _dot_t(o_ref[h].astype(BF16), whole(wo_ref, _ds(h * 2 * DH, 2 * DH)))

    def project_pair(h):
        attn_ref[...] += project(h) + project(h + 2)

    enqueue(keys(0, 4), [pltpu.make_async_copy(c_hbm, c_ref, sems.at[S_C]),
                         pltpu.make_async_copy(x_hbm, x_ref, sems.at[S_X])])
    _loop(0, 7, lambda i: enqueue(keys(4 + 8 * i, 8), wm_part(i)))

    def keys_and_wq(i):
        enqueue(keys(60 + 3 * i, 3), wide_part(wq_hbm, wq_ref, S_WQ, i))
        pl.when(i == 8)(condition)
    _loop(0, 22, keys_and_wq)
    enqueue(keys(126, 2), wide_part(wq_hbm, wq_ref, S_WQ, 22))
    _loop(0, 5, lambda i: enqueue(values(3 * i, 3), wide_part(wq_hbm, wq_ref, S_WQ, 23 + i)))

    def values_and_wo(i):
        enqueue(values(15 + 3 * i, 3), wide_part(wo_hbm, wo_ref, S_WO, i))
        n = (i - 5) >> 1

        @pl.when((i & 1) == 1)
        def _():
            pl.when(n == -1)(queries)
            pl.when((n >= 0) & (n < HKV))(lambda: scores(n))
            pl.when(n >= HKV)(lambda: context(((n & 1) << 1) + ((n >> 1) & 1)))
    _loop(0, 28, values_and_wo)

    enqueue(values(99, 1), [])

    def values_and_w3(i):
        enqueue(values(100 + 4 * i, 4), narrow_rows(w3_hbm, w3_ref, S_W3, 2 * i, FF_CUTS))

        @pl.when(i == 1)
        def _():
            landed(wo_ref, S_WO)
            attn_ref[...] = jnp.zeros((ROWS, D), F32)
        pl.when((i == 4) | (i == 5))(lambda: context(2 * i - 4))
        pl.when((i == 2) | (i == 3) | (i == 6))(lambda: project_pair(i - 2))
    _loop(0, 7, values_and_w3)

    w3 = narrow_rows(w3_hbm, w3_ref, S_W3, 14, END_CUTS * 7)
    w4 = narrow_rows(w4_hbm, w4_ref, S_W4, 0, END_CUTS * 10) + narrow_rows(w4_hbm, w4_ref, S_W4 + 1, 20, END_CUTS * 4)
    rest = [copy for j in range(21) for copy in (w3[2 * j], w3[2 * j + 1], w4[j])] + w4[21:]
    main, side = [copy for j, copy in enumerate(rest) if j % 3], rest[::3]
    for i, (r0, n) in enumerate(GATE_BLOCKS):
        for r in range(r0, r0 + n, 8):
            for half in ((slice(None),) if i == 0 else (0, 1)):
                at = (half, pl.ds(r, 8), pl.ds(LATE, 6 * D - LATE))
                main.append(pltpu.make_async_copy(wm_hbm.at[at], wm_ref.at[at], sems.at[S_GATE + i]))
    for j, copy in enumerate(main):
        copy.start(priority=1)
        if side and j >= 24 and j % 2 == 0:
            side.pop(0).start(priority=0)
        if j == 48:
            _loop(0, 2, lambda u: context(5 + 2 * u))
        if j == 60:
            attn = attn_ref[...] + project(5) + project(7)
            x = jnp.broadcast_to(x_ref[0].astype(F32), (ROWS, D))
            x = x + mod_ref[2] * (attn + pltpu.roll(attn, 1, 0))
            h_mlp = _layernorm(x) * (1.0 + mod_ref[4]) + mod_ref[3]
            normed = _layernorm(h_mlp).astype(BF16)
            mod_ref[0] = x
            mod_ref[1] = h_mlp
        if j == 90:
            landed(w3_ref, S_W3)
            hidden = jax.nn.gelu(_dot(normed, whole(w3_ref)), approximate=True).astype(BF16)
    assert not side

    landed(w4_ref.at[:, pl.ds(0, 160)], S_W4)
    y02 = _dot_t(hidden, jnp.concatenate([w4_ref[0, 0:128], w4_ref[1, 32:160]], axis=0))
    landed(w4_ref.at[:, pl.ds(160, 64)], S_W4 + 1)
    y13 = _dot_t(hidden, jnp.concatenate([w4_ref[0, 128:224], w4_ref[1, 0:32], w4_ref[1, 160:224]], axis=0))
    y = [y02[:, :128], y13[:, :128], y02[:, 128:], y13[:, 128:]]
    y = [part + mod_ref[1, :, t * 128:t * 128 + part.shape[1]] for t, part in enumerate(y)]

    sums = [jnp.zeros((ROWS, 128), F32)] * 3
    for i, (r0, n) in enumerate(GATE_BLOCKS):
        landed(wm_ref.at[:, pl.ds(r0, n), pl.ds(LATE, 6 * D - LATE)], S_GATE + i)
        for half in range(2):
            for r in range(r0, r0 + n, 16):
                c = cond_ref[half * D // 2 + r:half * D // 2 + r + 16, :]
                for t in range(3):
                    w = wm_ref[half, r:r + 16, LATE + t * 128:LATE + (t + 1) * 128].astype(F32) * c
                    sums[t] = sums[t] + (w[:8] + w[8:])
    low = lax.broadcasted_iota(jnp.int32, (1, 128), 1) < 64
    sums = [pltpu.roll(jnp.sum(s, axis=0, keepdims=True), 64, 1) for s in sums]
    gates = [jnp.where(low, a, b) for a, b in zip([mod_ref[5, 0:1, 0:128]] + sums[:2], sums)] + [sums[2][:, :64]]
    for t, (g, m) in enumerate(zip(gates, y)):
        cols = slice(t * 128, t * 128 + g.shape[1])
        out_ref[0, :, cols] = (mod_ref[0, 0:1, cols] + g * m[0:1]).astype(BF16)
    store = pltpu.make_async_copy(out_ref, out_hbm, sems.at[S_X])
    store.start()
    store.wait()


@jax.jit
def pallas_adaLN_cond__sliding_block_cached__mixer_s_mlp__decode_kernel(
    A_x: jax.Array,
    A_k_cache: jax.Array,
    A_v_cache: jax.Array,
    A_wq: jax.Array,
    A_wo: jax.Array,
    B_x: jax.Array,
    B_w1: jax.Array,
    B_w2: jax.Array,
    B_w3: jax.Array,
    B_w4: jax.Array,
    c: jax.Array,
    w_mod: jax.Array,
):
    keys = A_k_cache.shape[2]
    assert A_x.shape == (1, 1, D) and A_k_cache.shape == (1, HKV, keys, DH)
    assert min(4096, max(256, keys // 4)) == WINDOW and keys % (WINDOW // 2) == 0
    hbm = pl.BlockSpec(memory_space=pltpu.HBM)
    halves = lambda w: w.reshape(2, D // 2, w.shape[1])
    windows = lambda cache: cache.reshape(HKV, -1, WINDOW // 2, DH)
    return pl.pallas_call(
        _kernel,
        out_shape=jax.ShapeDtypeStruct(A_x.shape, A_x.dtype),
        in_specs=[hbm] * 9,
        out_specs=hbm,
        scratch_shapes=[
            pltpu.VMEM((1, 1, D), BF16),
            pltpu.VMEM((1, D), BF16),
            pltpu.VMEM((2, D // 2, 6 * D), BF16),
            pltpu.VMEM((2, D // 2, HQ * DH), BF16),
            pltpu.VMEM((HKV, 2, WINDOW // 2, DH), BF16),
            pltpu.VMEM((HKV, 2, WINDOW // 2, DH), BF16),
            pltpu.VMEM((2, D // 2, HQ * DH), BF16),
            pltpu.VMEM((2, D // 2, F), BF16),
            pltpu.VMEM((2, D // 2, F), BF16),
            pltpu.VMEM((512, 128), F32),
            pltpu.VMEM((HKV, ROWS, DH), F32),
            pltpu.VMEM((HKV, ROWS, WINDOW), F32),
            pltpu.VMEM((HKV, ROWS, 128), F32),
            pltpu.VMEM((HKV, ROWS, 2 * DH), F32),
            pltpu.VMEM((ROWS, D), F32),
            pltpu.VMEM((6, ROWS, D), F32),
            pltpu.VMEM((1, 1, D), BF16),
            pltpu.SemaphoreType.DMA((S_GATE + len(GATE_BLOCKS),)),
        ],
        compiler_params=pltpu.CompilerParams(
            vmem_limit_bytes=100 * 2**20,
            disable_semaphore_checks=True,
        ),
        name="adaln_decode",
    )(A_x, c, halves(w_mod), halves(A_wq), windows(A_k_cache), windows(A_v_cache), halves(A_wo.T),
      halves(B_w3), halves(B_w4.T))
```
